```python
import os as _os
_os.environ.setdefault("JAX_PLATFORMS", "cpu")
import jax
import jax.numpy as jnp

def _softmax(x, axis=-1):
    return jax.nn.softmax(x, axis=axis)
def _gelu(x):
    return jax.nn.gelu(x, approximate=True)
def _silu(x):
    return jax.nn.silu(x)
def _sigmoid(x):
    return jax.nn.sigmoid(x)
def _layernorm(x, axis=-1, eps=1e-5):
    m = jnp.mean(x, axis=axis, keepdims=True)
    v = jnp.var(x, axis=axis, keepdims=True)
    return (x - m) / jnp.sqrt(v + eps)
def _scatter_add(tgt, idx, src, axis=0):
    return tgt.at[idx].add(src)
def _segment_sum(src, seg, n):
    return jax.ops.segment_sum(src, seg, n)
class _Rng:
    def __init__(self, key):
        self._k = key
    def _next(self):
        self._k, sub = jax.random.split(self._k)
        return sub
    def normal(self, shape):
        return jax.random.normal(self._next(), shape, dtype=jnp.bfloat16)
    def randint(self, lo, hi, shape):
        return jax.random.randint(self._next(), shape, lo, hi, dtype=jnp.int32)
    def uniform(self, shape, lo=0.0, hi=1.0):
        return jax.random.uniform(self._next(), shape, jnp.bfloat16, lo, hi)
    def permutation(self, n):
        return jax.random.permutation(self._next(), n)


kernel_name = 'parallel_sum__softmax_full_mha__moe_arch_mod__prompt'

def setup_inputs():
    _rng = _Rng(jax.random.key(int.from_bytes(__import__("os").urandom(4), "little")))
    _w = (lambda a: (lambda t: t.astype(jnp.bfloat16) if jnp.issubdtype(t.dtype, jnp.floating) else t)(jnp.asarray(a)))
    def _A_setup():
        B, S, D = 1, 2048, 512
        return {
            "x": _w((lambda *s: _rng.normal(s) * 0.05)(B, S, D)),
            "wqkv": _w((lambda *s: _rng.normal(s) * 0.1)(D, 3 * D)),
            "wo": _w((lambda *s: _rng.normal(s) * 0.05)(D, D)),
        }
    _A_in = _A_setup()

    def _B_setup():
        B, S, D, F, C = 1, 2048, 512, 1792, 1
        return {
            "x": _w((lambda *s: _rng.normal(s) * 0.05)(B, S, D)),
            "w_r": _w((lambda *s: _rng.normal(s) * 1.6)(D)),
            "w_gate": _w((lambda *s: _rng.normal(s) * 0.1)(D, F)),
            "w_up": _w((lambda *s: _rng.normal(s) * 0.1)(D, F)),
            "w_down": _w((lambda *s: _rng.normal(s) * 0.1)(F, D)),
        }
    _B_in = _B_setup()

    return {
        "A_x": _A_in["x"],
        "A_wqkv": _A_in["wqkv"],
        "A_wo": _A_in["wo"],
        "B_x": _B_in["x"],
        "B_w_r": _B_in["w_r"],
        "B_w_gate": _B_in["w_gate"],
        "B_w_up": _B_in["w_up"],
        "B_w_down": _B_in["w_down"],
    }

def reference(A_x, A_wqkv, A_wo, B_x, B_w_r, B_w_gate, B_w_up, B_w_down):
    def _A_ref(x, wqkv, wo):
        B, S, D = x.shape
        H = 32; Dh = D // H
        qkv = (lambda x, *d: x.transpose(*d))((x @ wqkv).reshape(B, S, 3, H, Dh), 2, 0, 3, 1, 4)
        q, k, v = qkv[0], qkv[1], qkv[2]
        scale = Dh ** -0.5
        scores = jnp.einsum("bhqd,bhkd->bhqk", q, k) * scale
        p = _softmax(scores, axis=-1)
        o = jnp.einsum("bhqk,bhkd->bhqd", p, v)
        return (lambda x, *d: x.transpose(*d))(o, 0, 2, 1, 3).reshape(B, S, D) @ wo

    def _B_ref(x, w_r, w_gate, w_up, w_down):
        B, S, D = x.shape
        C = 1
        r = x @ w_r
        idx = jnp.argsort(-r, axis=-1)[:, :C]
        idx_e = jnp.repeat(idx.reshape(B, C, 1), D, axis=2)
        x_sel = jnp.take_along_axis(x, idx_e, axis=1)
        g = _silu(x_sel @ w_gate)
        u = x_sel @ w_up
        y = (g * u) @ w_down
        r_sel = _sigmoid(jnp.take_along_axis(r, idx, axis=1))
        y = y * r_sel.reshape(B, C, 1)
        b_off = (jnp.arange(B) * S).reshape(B, 1)
        flat_idx = (idx + b_off).reshape(B * C)
        zero = (x * 0.0).reshape(B * S, D)
        upd = _scatter_add(zero, flat_idx, y.reshape(B * C, D), axis=0)
        return x + upd.reshape(B, S, D)

    x = A_x
    xn = _layernorm(x, axis=-1)
    return x + _A_ref(xn, A_wqkv, A_wo) + _B_ref(xn, B_w_r, B_w_gate, B_w_up, B_w_down)
```

```python
import math

import jax
import jax.numpy as jnp
from jax import lax
import jax.experimental.pallas as pl
import jax.experimental.pallas.tpu as pltpu

F32 = jnp.float32
BF16 = jnp.bfloat16

S, D, H, DH, F = 2048, 512, 32, 16, 1792
EPS = 1e-5
BQ = 512
BK = 128
NK = S // BK
NQ = S // BQ
NT = H * NQ
LAG = 1
SUB = 32
RC = 512
NC = S // RC
QSCALE = (DH ** -0.5) * math.log2(math.e)

_NT_DIMS = (((1,), (1,)), ((), ()))
_TN_DIMS = (((0,), (0,)), ((), ()))


def _r16(a):
    return a.astype(BF16).astype(F32)


def _kernel(x_hbm, wqkv_hbm, wo_hbm, wr_ref, wg_hbm, wu_hbm, wd_hbm, out_hbm,
            x_v, wqkv_v, wo_v, wg_v, wu_v, wd_v, out_v,
            xn_v, wqvT_v, k_v, qT_v, vT_v, oT_v, sA, sB, upd_v,
            sem_x, sem_w, sem_o):
    def x_copy(c):
        return pltpu.make_async_copy(x_hbm.at[0, pl.ds(c * RC, RC)], x_v.at[pl.ds(c * RC, RC)], sem_x.at[c])

    w_copies = [pltpu.make_async_copy(s, d, sem_w.at[i]) for i, (s, d) in enumerate(
        [(wqkv_hbm, wqkv_v), (wo_hbm, wo_v), (wg_hbm, wg_v), (wu_hbm, wu_v), (wd_hbm, wd_v)])]

    def o_copy(qi, slot):
        return pltpu.make_async_copy(out_v.at[pl.ds(qi * BQ, BQ)], out_hbm.at[0, pl.ds(qi * BQ, BQ)], sem_o.at[slot])

    x_copy(0).start()
    w_copies[0].start()
    for c in range(1, NC):
        x_copy(c).start()

    wr = wr_ref[...].astype(F32)

    def layernorm(c):
        xc = x_v[pl.ds(c * RC, RC), :].astype(F32)
        mean = jnp.sum(xc, axis=1, keepdims=True) * (1.0 / D)
        cen = xc - mean
        var = jnp.sum(cen * cen, axis=1, keepdims=True) * (1.0 / D)
        d = _r16(xc - _r16(mean))
        sd = _r16(jnp.sqrt(_r16(_r16(var) + _r16(jnp.full((1, 1), EPS, F32)))))
        xn = (d * (1.0 / sd)).astype(BF16)
        xn_v[pl.ds(c * RC, RC), :] = xn
        r = _r16(jnp.sum(xn.astype(F32) * wr, axis=1, keepdims=True))
        rmax = jnp.max(r, axis=0, keepdims=True)
        rows = lax.broadcasted_iota(jnp.int32, (RC, 1), 0) + c * RC
        ridx = jnp.min(jnp.where(r == rmax, rows, S - 1), axis=0, keepdims=True)
        return xn, rmax, ridx

    def project(c, xn):
        k = jnp.dot(xn, wqkv_v[:, D:2 * D], preferred_element_type=F32).astype(BF16)
        for g in range(D // 128):
            k_v[g, pl.ds(c * RC, RC), :] = k[:, g * 128:(g + 1) * 128]
        qv = lax.dot_general(wqvT_v[...], xn, _NT_DIMS, preferred_element_type=F32)
        qT_v[:, pl.ds(c * RC, RC)] = (qv[:D] * QSCALE).astype(BF16)
        vT_v[:, pl.ds(c * RC, RC)] = qv[D:].astype(BF16)

    x_copy(0).wait()
    xn_c, best_r, best_i = layernorm(0)
    w_copies[0].wait()
    for i in range(1, 5):
        w_copies[i].start()
    wqvT_v[0:D, :] = wqkv_v[:, 0:D].astype(F32).T.astype(BF16)
    wqvT_v[D:2 * D, :] = wqkv_v[:, 2 * D:3 * D].astype(F32).T.astype(BF16)
    for c in range(NC):
        if c + 1 < NC:
            x_copy(c + 1).wait()
            xn_n, r_n, i_n = layernorm(c + 1)
            better = r_n > best_r
            best_r = jnp.where(better, r_n, best_r)
            best_i = jnp.where(better, i_n, best_i)
        project(c, xn_c)
        if c + 1 < NC:
            xn_c = xn_n

    for i in range(1, 5):
        w_copies[i].wait()
    idx = jnp.clip(jnp.max(best_i), 0, S - 1)
    base = pl.multiple_of((idx // 16) * 16, 16)
    xs = xn_v[pl.ds(base, 16), :]
    gate = jnp.dot(xs, wg_v[...], preferred_element_type=F32)
    up = jnp.dot(xs, wu_v[...], preferred_element_type=F32)
    hid = (gate * jax.nn.sigmoid(gate) * up).astype(BF16)
    y = jnp.dot(hid, wd_v[...], preferred_element_type=F32) * jax.nn.sigmoid(best_r)
    sel = lax.broadcasted_iota(jnp.int32, (16, 1), 0) == (idx - base)
    upd_v[...] = jnp.broadcast_to(jnp.sum(jnp.where(sel, y, 0.0), axis=0, keepdims=True), (8, D))

    bufs = (sA, sB)

    def hq(t):
        return t % H, t // H

    def mkw(t):
        h, qi = hq(t)
        qh = qT_v[pl.ds(pl.multiple_of(h * DH, DH), DH), pl.ds(pl.multiple_of(qi * BQ, BQ), BQ)]
        z = jnp.zeros_like(qh)
        hm = h % 8
        return jnp.concatenate([jnp.where(hm == i, qh, z) for i in range(8)], axis=0)

    def qk(t, w, j, m8, sref):
        h, _ = hq(t)
        s = jnp.dot(k_v[h // 8, j * BK:(j + 1) * BK, :], w, preferred_element_type=F32)
        sref[j * BK:(j + 1) * BK, :] = s
        mx = jnp.max(s.reshape(BK // 8, 8, BQ), axis=0)
        return mx if m8 is None else jnp.maximum(m8, mx)

    def pv(t, m, j, l8, acc, sref):
        h, _ = hq(t)
        ls = None
        ps = []
        for r in range(BK // SUB):
            p = jnp.exp2(sref[j * BK + r * SUB:j * BK + (r + 1) * SUB, :] - m)
            l1 = jnp.sum(p.reshape(SUB // 8, 8, BQ), axis=0)
            ls = l1 if ls is None else ls + l1
            ps.append(p.astype(BF16))
        pb = jnp.concatenate(ps, axis=0)
        vh = vT_v[pl.ds(pl.multiple_of(h * DH, DH), DH), j * BK:(j + 1) * BK]
        r = jnp.dot(vh, pb, preferred_element_type=F32)
        return (ls, r) if l8 is None else (l8 + ls, acc + r)

    def fin(t, l8, acc):
        h, qi = hq(t)
        l = jnp.sum(l8, axis=0, keepdims=True)
        oT_v[pl.ds(pl.multiple_of(h * DH, DH), DH), pl.ds(pl.multiple_of(qi * BQ, BQ), BQ)] = (acc / l).astype(BF16)

    def mfin(m8):
        return jnp.max(m8, axis=0, keepdims=True)

    def out_proj(qi, slot):
        q0 = pl.multiple_of(qi * BQ, BQ)
        y = lax.dot_general(oT_v[:, pl.ds(q0, BQ)], wo_v[...], _TN_DIMS, preferred_element_type=F32)
        res = x_v[pl.ds(q0, BQ), :].astype(F32) + xn_v[pl.ds(q0, BQ), :].astype(F32)
        rows = lax.broadcasted_iota(jnp.int32, (BQ, 1), 0) + q0
        res = res + jnp.where(rows == idx, upd_v[0:1, :], 0.0)
        out_v[pl.ds(q0, BQ), :] = (res + y).astype(BF16)
        o_copy(qi, slot).start()

    U = 2
    NB = NT // U

    def body(b, carry, first=False, last=False):
        m_cur, m_prev, l8p, accp = carry
        ms = {0: m_cur, -1: m_prev}
        st = {-1: (l8p, accp)}
        m8 = w = None
        nsteps = U * NK
        for s in range(nsteps + (LAG if last else 0)):
            i, j = divmod(s, NK)
            ip, jp = divmod(s - LAG, NK)
            if s < nsteps and not (last and i == U - 1):
                t = b * U + i + 1
                if j == 0:
                    w, m8 = mkw(t), None
                m8 = qk(t, w, j, m8, bufs[(i + 1) % 2])
                if j == NK - 1:
                    ms[i + 1] = mfin(m8)
            if not (first and ip < 0):
                t = b * U + ip
                l8, acc = st.get(ip, (None, None))
                l8, acc = pv(t, ms[ip], jp, l8, acc, bufs[ip % 2])
                st[ip] = (l8, acc)
                if jp == NK - 1:
                    fin(t, l8, acc)
        if last:
            return None
        l8, acc = st[U - 1]
        return ms[U], ms[U - 1], l8, acc

    w0, m8 = mkw(0), None
    for j in range(NK):
        m8 = qk(0, w0, j, m8, sA)
    m_first = mfin(m8)
    carry = body(0, (m_first, m_first, jnp.zeros((8, BQ), F32), jnp.zeros((DH, BQ), F32)), first=True)

    per_q = H // U

    def loop_body(b, carry):
        carry = body(b, carry)

        @pl.when(b % per_q == 0)
        def _():
            out_proj(b // per_q - 1, b // per_q - 1)

        return carry

    carry = lax.fori_loop(1, NB - 1, loop_body, carry)
    body(NB - 1, carry, last=True)
    out_proj(NQ - 1, NQ - 1)
    for qi in range(NQ):
        o_copy(qi, qi).wait()


@jax.jit
def pallas_parallel_sum__softmax_full_mha__moe_arch_mod__prompt_kernel(
    A_x: jax.Array,
    A_wqkv: jax.Array,
    A_wo: jax.Array,
    B_x: jax.Array,
    B_w_r: jax.Array,
    B_w_gate: jax.Array,
    B_w_up: jax.Array,
    B_w_down: jax.Array,
):
    del B_x
    hbm = pl.BlockSpec(memory_space=pl.ANY)
    vm = pltpu.VMEM
    return pl.pallas_call(
        _kernel,
        out_shape=jax.ShapeDtypeStruct((1, S, D), BF16),
        in_specs=[hbm, hbm, hbm, pl.BlockSpec(memory_space=pltpu.VMEM), hbm, hbm, hbm],
        out_specs=hbm,
        scratch_shapes=[
            vm((S, D), BF16), vm((D, 3 * D), BF16), vm((D, D), BF16),
            vm((D, F), BF16), vm((D, F), BF16), vm((F, D), BF16), vm((S, D), BF16),
            vm((S, D), BF16), vm((2 * D, D), BF16), vm((D // 128, S, 128), BF16),
            vm((D, S), BF16), vm((D, S), BF16), vm((D, S), BF16),
            vm((S, BQ), F32), vm((S, BQ), F32), vm((8, D), F32),
            pltpu.SemaphoreType.DMA((NC,)), pltpu.SemaphoreType.DMA((5,)), pltpu.SemaphoreType.DMA((NQ,)),
        ],
        compiler_params=pltpu.CompilerParams(vmem_limit_bytes=100 * 2 ** 20),
    )(A_x, A_wqkv, A_wo, B_w_r.reshape(1, D), B_w_gate, B_w_up, B_w_down)
```

```python
import math

import jax
import jax.numpy as jnp
from jax import lax
import jax.experimental.pallas as pl
import jax.experimental.pallas.tpu as pltpu

F32 = jnp.float32
BF16 = jnp.bfloat16

S, D, H, DH, F = 2048, 512, 32, 16, 1792
EPS = 1e-5
BQ = 512
BK = 128
NK = S // BK
NQ = S // BQ
NT = H * NQ
LAG = 1
SUB = 32
DEPD, DEPG = 3, 15
U0, U, U1 = 6, 8, 2
MB = 256
LP = 64
P0 = 256
OP = 256
RC = 512
QSCALE = (DH ** -0.5) * math.log2(math.e)

_NT_DIMS = (((1,), (1,)), ((), ()))
_TN_DIMS = (((0,), (0,)), ((), ()))


def _r16(a):
    return a.astype(BF16).astype(F32)


def _kernel(x_hbm, wqkv_hbm, wo_hbm, wr_ref, wg_hbm, wu_hbm, wd_hbm, out_hbm,
            x_v, wqkv_v, wo_v, wg_v, wu_v, wd_v, out_v,
            xn_v, wqvT_v, k_v, qT_v, vT_v, oT_v, sA, sB, upd_v, part_v,
            sem_x, sem_w, sem_o):
    def x_copy(i, r0, n):
        return pltpu.make_async_copy(x_hbm.at[0, pl.ds(r0, n)], x_v.at[pl.ds(r0, n)], sem_x.at[i])

    def wcol_copy(i):
        return pltpu.make_async_copy(wqkv_hbm.at[:, pl.ds(i * D, D)], wqkv_v.at[:, pl.ds(i * D, D)], sem_w.at[i])

    late = [pltpu.make_async_copy(s_, d_, sem_w.at[3 + i]) for i, (s_, d_) in enumerate(
        [(wo_hbm, wo_v), (wg_hbm, wg_v), (wu_hbm, wu_v), (wd_hbm, wd_v)])]

    NP = BQ // OP

    def o_copy(qi, p):
        r0 = qi * BQ + p * OP
        return pltpu.make_async_copy(out_v.at[pl.ds(r0, OP)], out_hbm.at[0, pl.ds(r0, OP)], sem_o.at[qi * NP + p])

    cps = {'0': x_copy(0, 0, P0), '1': x_copy(1, P0, 1024 - P0), '2': x_copy(2, 1024, 512), '3': x_copy(3, 1536, 512),
           'q': wcol_copy(0), 'k': wcol_copy(1), 'v': wcol_copy(2)}
    for ch in '0k1qv23':
        cps[ch].start()

    wr = wr_ref[...].astype(F32).reshape(1, D)
    best = [None, None]

    def after(val, dep):
        return val if dep is None else jnp.where(dep == dep, val, dep)

    def layernorm(r0, n, dep=None):
        xc = x_v[pl.ds(r0, n), :].astype(F32)
        inv = after(jnp.full((8, 128), 1.0 / D, F32), dep)[:, 0:1]
        mean = (jnp.sum(xc, axis=1, keepdims=True).reshape(n // 8, 8, 1) * inv[None]).reshape(n, 1)
        cen = xc - mean
        var = jnp.sum(cen * cen, axis=1, keepdims=True) * (1.0 / D)
        d = _r16(xc - _r16(mean))
        ve = _r16(_r16(var) + _r16(jnp.full((1, 1), EPS, F32)))
        sd = _r16(jnp.sqrt(ve))
        r0_ = pl.reciprocal(sd, approx=True)
        rinv = jnp.where(sd == jnp.inf, 0.0, r0_ * (2.0 - sd * r0_))
        xn = (d * rinv).astype(BF16)
        xn_v[pl.ds(r0, n), :] = xn
        r = _r16(jnp.sum(xn.astype(F32) * wr, axis=1, keepdims=True))
        rmax = jnp.max(r, axis=0, keepdims=True)
        rows = lax.broadcasted_iota(jnp.int32, (n, 1), 0) + r0
        ridx = jnp.min(jnp.where(r == rmax, rows, S - 1), axis=0, keepdims=True)
        if best[0] is None:
            best[0], best[1] = rmax, ridx
        else:
            better = rmax > best[0]
            best[0], best[1] = jnp.where(better, rmax, best[0]), jnp.where(better, ridx, best[1])

    def k_dots(lo, hi):
        for r0 in range(lo, hi, MB):
            k = jnp.dot(xn_v[pl.ds(r0, MB), :], wqkv_v[:, D:2 * D], preferred_element_type=F32)
            kb = k.astype(BF16)
            for g in range(D // 128):
                k_v[g, pl.ds(r0, MB), :] = kb[:, g * 128:(g + 1) * 128]
            yield k[0:8, 0:128]

    def qv_dots(c):
        xn = xn_v[pl.ds(c * RC, RC), :]
        for r0 in range(0, 2 * D, MB):
            qv = lax.dot_general(wqvT_v[pl.ds(r0, MB), :], xn, _NT_DIMS, preferred_element_type=F32)
            if r0 < D:
                qT_v[pl.ds(r0, MB), pl.ds(c * RC, RC)] = (qv * QSCALE).astype(BF16)
            else:
                vT_v[pl.ds(r0 - D, MB), pl.ds(c * RC, RC)] = qv.astype(BF16)
            yield qv[0:8, 0:128]

    last_ev = [None]

    def run(gens, fillers):
        n_ev = sum(n for n, _ in gens)
        done = k = 0
        for _, g in gens:
            for d in g:
                done += 1
                while k < len(fillers) and k * n_ev < done * len(fillers):
                    fillers[k](last_ev[0])
                    k += 1
                last_ev[0] = d

    nk_, nqv_ = RC // MB, 2 * D // MB

    def ln_fill(lo, hi):
        return [(lambda dep, r0=r0: layernorm(r0, LP, dep)) for r0 in range(lo, hi, LP)]

    def transpose_fill():
        def job(i, r0):
            def f(dep):
                wqvT_v[pl.ds(i * D + r0, 128), :] = wqkv_v[:, pl.ds(2 * i * D + r0, 128)].astype(F32).T.astype(BF16)
            return f
        return [job(i, r0) for i in range(2) for r0 in range(0, D, 128)]

    ffn = {}

    def ffn_fill():
        def start(dep):
            idx = jnp.clip(jnp.max(best[1]), 0, S - 1)
            base = pl.multiple_of((idx // 16) * 16, 16)
            ffn['idx'], ffn['base'] = idx, base
            ffn['xs'] = xn_v[pl.ds(base, 16), :]
            ffn['hid'] = []
            ffn['y'] = None
        def gu(i):
            def job(dep):
                cols = pl.ds(i * 256, 256)
                gate = jnp.dot(ffn['xs'], wg_v[:, cols], preferred_element_type=F32)
                up = jnp.dot(ffn['xs'], wu_v[:, cols], preferred_element_type=F32)
                ffn['hid'].append((gate * jax.nn.sigmoid(gate) * up).astype(BF16))
            return job
        def dn(i):
            def job(dep):
                y = jnp.dot(ffn['hid'][i], wd_v[pl.ds(i * 256, 256), :], preferred_element_type=F32)
                ffn['y'] = y if ffn['y'] is None else ffn['y'] + y
            return job
        def end(dep):
            y = ffn['y'] * jax.nn.sigmoid(best[0])
            sel = lax.broadcasted_iota(jnp.int32, (16, 1), 0) == (ffn['idx'] - ffn['base'])
            upd_v[...] = jnp.broadcast_to(jnp.sum(jnp.where(sel, y, 0.0), axis=0, keepdims=True), (8, D))
        n = F // 256
        return [start] + [gu(i) for i in range(n)] + [dn(i) for i in range(n)] + [end]

    cps['0'].wait()
    for f in ln_fill(0, P0):
        f(None)
    cps['k'].wait()
    cps['1'].wait()
    for r0 in range(0, 1024 - MB, MB):
        run([(1, k_dots(r0, r0 + MB))], ln_fill(max(P0, r0 + MB), r0 + 2 * MB))
    for ch in 'qv23':
        cps[ch].wait()
    for cp in late:
        cp.start()
    run([(1, k_dots(1024 - MB, 1024))], transpose_fill())
    run([(nqv_, qv_dots(0))], ln_fill(1024, 1536))
    run([(nqv_, qv_dots(1))], ln_fill(1536, 2048))
    run([(nk_, k_dots(1024, 1536))], [])
    for cp in late:
        cp.wait()
    run([(nqv_, qv_dots(2)), (nk_, k_dots(1536, 2048)), (nqv_, qv_dots(3))], ffn_fill())
    idx = ffn['idx']
    bufs = (sA, sB)

    def hq(t):
        return t % H, t // H

    def mkw(t, hs=None):
        h, qi = hq(t)
        qh = qT_v[pl.ds(pl.multiple_of(h * DH, DH), DH), pl.ds(pl.multiple_of(qi * BQ, BQ), BQ)]
        z = jnp.zeros_like(qh)
        if isinstance(h, int):
            hs = h % 8
        assert hs is not None
        return jnp.concatenate([qh if i == hs else z for i in range(8)], axis=0)


    def qk(t, w, j, m8, sref):
        h, _ = hq(t)
        s = jnp.dot(k_v[h // 8, j * BK:(j + 1) * BK, :], w, preferred_element_type=F32)
        sref[j * BK:(j + 1) * BK, :] = s
        mx = jnp.max(s.reshape(BK // 8, 8, BQ), axis=0)
        return (mx if m8 is None else jnp.maximum(m8, mx)), s

    def pv(t, m, j, l8, acc, sref):
        h, _ = hq(t)
        ps = []
        for r in range(BK // SUB):
            sv = sref[j * BK + r * SUB:j * BK + (r + 1) * SUB, :]
            if m.shape[0] == 8:
                p = jnp.exp2(sv.reshape(SUB // 8, 8, BQ) - m[None]).reshape(SUB, BQ)
            else:
                p = jnp.exp2(sv - m)
            l1 = jnp.sum(p.reshape(SUB // 8, 8, BQ), axis=0)
            l8 = l1 if l8 is None else l8 + l1
            ps.append(p)
        pb = jnp.concatenate(ps, axis=0).astype(BF16)
        vh = vT_v[pl.ds(pl.multiple_of(h * DH, DH), DH), j * BK:(j + 1) * BK]
        r = jnp.dot(vh, pb, preferred_element_type=F32)
        return l8, (r if acc is None else acc + r)

    def fin(t, l8, acc):
        h, qi = hq(t)
        l = jnp.sum(l8, axis=0, keepdims=True)
        oT_v[pl.ds(pl.multiple_of(h * DH, DH), DH), pl.ds(pl.multiple_of(qi * BQ, BQ), BQ)] = (acc / l).astype(BF16)

    def mfin(m8):
        return jnp.max(m8, axis=0, keepdims=True)

    def residual(q0):
        res = x_v[pl.ds(q0, OP), :].astype(F32) + xn_v[pl.ds(q0, OP), :].astype(F32)
        rows = lax.broadcasted_iota(jnp.int32, (OP, 1), 0) + q0
        return res + jnp.where(rows == idx, upd_v[0:1, :], 0.0)

    def proj(q0, k0, k1):
        return lax.dot_general(oT_v[k0:k1, pl.ds(q0, OP)], wo_v[k0:k1, :], _TN_DIMS, preferred_element_type=F32)

    def out_proj(qi):
        for p in range(NP):
            q0 = qi * BQ + p * OP
            out_v[pl.ds(q0, OP), :] = (residual(q0) + proj(q0, 0, D)).astype(BF16)
            o_copy(qi, p).start()

    KS = D - 128

    def tail_part(p, k0):
        q0 = S - BQ + p * OP
        y = proj(q0, k0, k0 + 128)
        part_v[p * OP:(p + 1) * OP, :] = (residual(q0) if k0 == 0 else part_v[p * OP:(p + 1) * OP, :]) + y

    tail_jobs = [(p, k0) for k0 in range(0, KS, 128) for p in range(NP)]

    def out_proj_last():
        for p in range(NP):
            q0 = S - BQ + p * OP
            out_v[pl.ds(q0, OP), :] = (part_v[p * OP:(p + 1) * OP, :] + proj(q0, KS, D)).astype(BF16)
            o_copy(NQ - 1, p).start()


    def body(t0, U, carry, first=False, last=False):
        m_cur, m_prev, l8p, accp = carry
        ms = {0: m_cur, -1: m_prev}
        st = {-1: (l8p, accp)}
        m8 = w = None
        nsteps = U * NK
        hist = {}
        for s in range(nsteps + (LAG if last else 0)):
            i, j = divmod(s, NK)
            ip, jp = divmod(s - LAG, NK)
            if last and s >= (U - 1) * NK:
                for n, job in enumerate(tail_jobs):
                    if n * NK // len(tail_jobs) == s - (U - 1) * NK:
                        tail_part(*job)
            if s < nsteps and not (last and i == U - 1):
                t = t0 + i + 1
                if j == 0:
                    w, m8 = mkw(t, (U0 + i + 1) % 8 if not (first or last) else None), None
                m8, hist[s] = qk(t, w, j, m8, bufs[(i + 1) % 2])
                if j == NK - 1:
                    ms[i + 1] = mfin(m8)
            if not (first and ip < 0):
                t = t0 + ip
                l8, acc = st.get(ip, (None, None))
                m = ms[ip]
                if (s - DEPD) in hist:
                    m = after(m, hist[s - DEPD][DEPG * 8:DEPG * 8 + 8])
                l8, acc = pv(t, m, jp, l8, acc, bufs[ip % 2])
                st[ip] = (l8, acc)
                if jp == NK - 1:
                    fin(t, l8, acc)
        if last:
            return None
        l8, acc = st[U - 1]
        return ms[U], ms[U - 1], l8, acc

    w0, m8 = mkw(0), None
    for j in range(NK):
        m8, _ = qk(0, w0, j, m8, sA)
    m_first = mfin(m8)
    carry = body(0, U0, (m_first, m_first, jnp.zeros((8, BQ), F32), jnp.zeros((DH, BQ), F32)), first=True)
    nloop = (NT - U0 - U1) // U
    assert U0 + U1 + nloop * U == NT and U % 8 == 0

    def loop_body(b, carry):
        return body(U0 + b * U, U, carry)

    carry = lax.fori_loop(0, nloop, loop_body, carry)
    body(NT - U1, U1, carry, last=True)
    for qi in range(NQ - 1):
        out_proj(qi)
    out_proj_last()
    for qi in range(NQ):
        for p in range(NP):
            o_copy(qi, p).wait()


@jax.jit
def pallas_parallel_sum__softmax_full_mha__moe_arch_mod__prompt_kernel(
    A_x: jax.Array,
    A_wqkv: jax.Array,
    A_wo: jax.Array,
    B_x: jax.Array,
    B_w_r: jax.Array,
    B_w_gate: jax.Array,
    B_w_up: jax.Array,
    B_w_down: jax.Array,
):
    del B_x
    hbm = pl.BlockSpec(memory_space=pl.ANY)
    vm = pltpu.VMEM
    return pl.pallas_call(
        _kernel,
        out_shape=jax.ShapeDtypeStruct((1, S, D), BF16),
        in_specs=[hbm, hbm, hbm, pl.BlockSpec(memory_space=pltpu.VMEM), hbm, hbm, hbm],
        out_specs=hbm,
        scratch_shapes=[
            vm((S, D), BF16), vm((D, 3 * D), BF16), vm((D, D), BF16),
            vm((D, F), BF16), vm((D, F), BF16), vm((F, D), BF16), vm((S, D), BF16),
            vm((S, D), BF16), vm((2 * D, D), BF16), vm((D // 128, S, 128), BF16),
            vm((D, S), BF16), vm((D, S), BF16), vm((D, S), BF16),
            vm((S, BQ), F32), vm((S, BQ), F32), vm((8, D), F32), vm((BQ, D), F32),
            pltpu.SemaphoreType.DMA((4,)), pltpu.SemaphoreType.DMA((7,)), pltpu.SemaphoreType.DMA((S // OP,)),
        ],
        compiler_params=pltpu.CompilerParams(vmem_limit_bytes=100 * 2 ** 20),
    )(A_x, A_wqkv, A_wo, B_w_r, B_w_gate, B_w_up, B_w_down)
```
